```python
import os as _os
_os.environ.setdefault("JAX_PLATFORMS", "cpu")
import jax
import jax.numpy as jnp

def _softmax(x, axis=-1):
    return jax.nn.softmax(x, axis=axis)
def _gelu(x):
    return jax.nn.gelu(x, approximate=True)
def _silu(x):
    return jax.nn.silu(x)
def _sigmoid(x):
    return jax.nn.sigmoid(x)
def _layernorm(x, axis=-1, eps=1e-5):
    m = jnp.mean(x, axis=axis, keepdims=True)
    v = jnp.var(x, axis=axis, keepdims=True)
    return (x - m) / jnp.sqrt(v + eps)
def _scatter_add(tgt, idx, src, axis=0):
    return tgt.at[idx].add(src)
def _segment_sum(src, seg, n):
    return jax.ops.segment_sum(src, seg, n)
class _Rng:
    def __init__(self, key):
        self._k = key
    def _next(self):
        self._k, sub = jax.random.split(self._k)
        return sub
    def normal(self, shape):
        return jax.random.normal(self._next(), shape, dtype=jnp.bfloat16)
    def randint(self, lo, hi, shape):
        return jax.random.randint(self._next(), shape, lo, hi, dtype=jnp.int32)
    def uniform(self, shape, lo=0.0, hi=1.0):
        return jax.random.uniform(self._next(), shape, jnp.bfloat16, lo, hi)
    def permutation(self, n):
        return jax.random.permutation(self._next(), n)


kernel_name = 'concat_heads__gqa_block_cached__mha_block_cached__near_ridge'

def setup_inputs():
    _rng = _Rng(jax.random.key(int.from_bytes(__import__("os").urandom(4), "little")))
    _w = (lambda a: (lambda t: t.astype(jnp.bfloat16) if jnp.issubdtype(t.dtype, jnp.floating) else t)(jnp.asarray(a)))
    def _A_setup():
        B, Sq, D = 16, 32, 512
        Hq, Hkv, Sk, Dh = 32, 8, 512, 128
        assert Hq % Hkv == 0, (Hq, Hkv)
        return {
            "x": _w((lambda *s: _rng.normal(s) * 0.8)(B, Sq, D)),
            "k_cache": _w((lambda *s: _rng.normal(s) * 0.8)(B, Hkv, Sk, Dh)),
            "v_cache": _w((lambda *s: _rng.normal(s) * 0.05)(B, Hkv, Sk, Dh)),
            "wq": _w((lambda *s: _rng.normal(s) * 0.8)(D, Hq * Dh) * (D ** -0.5)),
            "wo": _w((lambda *s: _rng.normal(s) * 0.05)(Hq * Dh, D) * ((Hq * Dh) ** -0.5)),
        }
    _A_in = _A_setup()

    def _B_setup():
        B, Sq, D = 16, 32, 512
        H, Sk, Dh = 32, 512, 128
        return {
            "x": _w((lambda *s: _rng.normal(s) * 0.8)(B, Sq, D)),
            "k_cache": _w((lambda *s: _rng.normal(s) * 0.8)(B, H, Sk, Dh)),
            "v_cache": _w((lambda *s: _rng.normal(s) * 0.05)(B, H, Sk, Dh)),
            "wq": _w((lambda *s: _rng.normal(s) * 0.8)(D, H * Dh) * (D ** -0.5)),
            "wo": _w((lambda *s: _rng.normal(s) * 0.05)(H * Dh, D) * ((H * Dh) ** -0.5)),
        }
    _B_in = _B_setup()

    return {
        "A_x": _A_in["x"],
        "A_k_cache": _A_in["k_cache"],
        "A_v_cache": _A_in["v_cache"],
        "A_wq": _A_in["wq"],
        "A_wo": _A_in["wo"],
        "B_x": _B_in["x"],
        "B_k_cache": _B_in["k_cache"],
        "B_v_cache": _B_in["v_cache"],
        "B_wq": _B_in["wq"],
        "B_wo": _B_in["wo"],
    }

def reference(A_x, A_k_cache, A_v_cache, A_wq, A_wo, B_x, B_k_cache, B_v_cache, B_wq, B_wo):
    def _A_ref(x, k_cache, v_cache, wq, wo):
        B, Sq, D = x.shape
        Hq, Dh = 32, 128
        Hkv = k_cache.shape[1]
        rep = Hq // Hkv
        q = (lambda x, *d: x.transpose(*d))((x @ wq).reshape(B, Sq, Hq, Dh), 0, 2, 1, 3)
        k = jnp.repeat(k_cache, rep, axis=1)
        v = jnp.repeat(v_cache, rep, axis=1)
        scores = jnp.einsum("bhqd,bhkd->bhqk", q, k) * (Dh ** -0.5)
        p = _softmax(scores, axis=-1)
        o = jnp.einsum("bhqk,bhkd->bhqd", p, v)
        return (lambda x, *d: x.transpose(*d))(o, 0, 2, 1, 3).reshape(B, Sq, Hq * Dh) @ wo

    def _B_ref(x, k_cache, v_cache, wq, wo):
        B, Sq, D = x.shape
        H, Dh = 32, 128
        q = (lambda x, *d: x.transpose(*d))((x @ wq).reshape(B, Sq, H, Dh), 0, 2, 1, 3)
        scores = jnp.einsum("bhqd,bhkd->bhqk", q, k_cache) * (Dh ** -0.5)
        p = _softmax(scores, axis=-1)
        o = jnp.einsum("bhqk,bhkd->bhqd", p, v_cache)
        return (lambda x, *d: x.transpose(*d))(o, 0, 2, 1, 3).reshape(B, Sq, H * Dh) @ wo

    a = _A_ref(A_x, A_k_cache, A_v_cache, A_wq, A_wo)
    b = _B_ref(B_x, B_k_cache, B_v_cache, B_wq, B_wo)
    return jnp.concatenate([a, b], axis=-1)
```

```python
import math

import jax
import jax.numpy as jnp
from jax import lax
import jax.experimental.pallas as pl
import jax.experimental.pallas.tpu as pltpu

B, SQ, D = 16, 32, 512
HQ, SK, DH = 32, 512, 128
REP = 4
ROWS = B * SQ
QSCALE = (DH ** -0.5) * math.log2(math.e)

CH = 128
NCH = SK // CH
UB = 4
UPH = B // UB
NU = HQ * UPH

DIST = 6
LAST_HEADS = 2
DIST_END = 3
NA = DIST + 1
NB = (DIST + UPH - 1) // UPH + 1
NMAIN = NU - UPH * LAST_HEADS
T0 = NMAIN - DIST
NHALF = 2 * UPH * LAST_HEADS
TEND = NU - 1 - DIST_END
NSLOW = 2 * (TEND - T0 + 1) - NHALF
BATCH_ORDER = tuple(range(0, B, 2)) + tuple(range(1, B, 2))


def _aligned(x, n):
    return x if isinstance(x, int) else pl.multiple_of(x, n)


def _start(copies):
    for n, (src, dst, sem) in enumerate(copies):
        pltpu.make_async_copy(src, dst, sem).start(priority=n % 2)


def _wait_total(like, sem):
    pltpu.make_async_copy(like, like, sem).wait()


def _mm(a, b):
    return jnp.dot(a, b, preferred_element_type=jnp.float32)


def _mm_nt(a, b):
    return lax.dot_general(a, b, (((1,), (1,)), ((), ())), preferred_element_type=jnp.float32)


def _softmax_parts(s):
    e = jnp.exp2(s - jnp.max(s, axis=1, keepdims=True))
    return e.astype(jnp.bfloat16), 1.0 / jnp.sum(e, axis=1, keepdims=True)


def _kernel(ax, ak, av, awq, awo, bx, bk, bv, bwq, bwo, out,
            x_buf, wq_buf, wo_buf, kv_buf, acc, stage, kv_sem, pro_sem, out_sem):
    bf16 = jnp.bfloat16
    kv_words = kv_buf.bitcast(jnp.uint32)

    def piece_b(slot, kv, b):
        return (slot * 2 + kv) * B + b

    def piece_a(slot, kv):
        return NB * 2 * B + slot * 2 + kv

    def load_piece(i):
        return pltpu.bitcast(kv_words[i], bf16)

    def copies_gqa(n):
        g, b, slot = n // B, n % B, n % NA
        return [(src.at[b, g, pl.ds(s * CH, CH)],
                 kv_buf.at[piece_a(slot, kv), pl.ds(s * CH, CH)],
                 kv_sem.at[NB + slot])
                for s in range(NCH) for kv, src in enumerate((ak, av))]

    def copies_mha(n):
        h = n // UPH
        slot = h % NB
        keys = pl.ds(_aligned((n % UPH) * CH, CH), CH)
        return [(src.at[b, h, keys], kv_buf.at[piece_b(slot, kv, b), keys], kv_sem.at[slot])
                for kv, src in enumerate((bk, bv)) for b in BATCH_ORDER]

    def start_unit_reads(n, carry):
        gqa, mha = copies_gqa(n), copies_mha(n)
        copies = []
        for i in range(4):
            copies += mha[8 * i:8 * i + 8] + gqa[2 * i:2 * i + 2]
        _start(copies)
        return carry

    def start_half_unit_reads(i, carry):
        j = i // 2
        h, b0 = HQ - LAST_HEADS + j // UPH, (j % UPH) * UB
        slot = h % NB
        copies = []
        for s in range(NCH // 2):
            keys = pl.ds(_aligned(((i % 2) * (NCH // 2) + s) * CH, CH), CH)
            copies += [(src.at[b0 + b, h, keys], kv_buf.at[piece_b(slot, kv, b0 + b), keys],
                        kv_sem.at[NB + NA + j])
                       for kv, src in enumerate((bk, bv)) for b in range(UB)]
        _start(copies)
        return carry

    def start_weight_reads(i, carry):
        copies = []
        for j in range(4):
            n = j * 32 + i
            rows, cols = pl.ds(_aligned((n // 2) * 8, 8), 8), pl.ds(_aligned((n % 2) * 2048, 2048), 2048)
            copies += [(w.at[rows, cols], wq_buf.at[part, rows, cols], pro_sem.at[1])
                       for part, w in enumerate((awq, bwq))]
        _start(copies)
        copies = []
        for j in range(4):
            rows = pl.ds(_aligned((j * 32 + i) * 32, 32), 32)
            copies += [(w.at[rows], wo_buf.at[part, rows], pro_sem.at[2])
                       for part, w in enumerate((awo, bwo))]
        _start(copies)
        return carry

    def start_writes(q, carry):
        _start([(stage.at[q * UB + b, pl.ds(j * 16, 16)], out.at[q * UB + b, pl.ds(j * 16, 16)], out_sem)
                for j in range(SQ // 16) for b in range(UB)])
        return carry

    def halves_before(u):
        return jnp.clip(u - T0, 0, NSLOW) + jnp.clip(2 * (u - T0 - NSLOW), 0, NHALF - NSLOW)

    def compute_unit(u):
        h, b0 = u // UPH, (u % UPH) * UB
        g, ba = u // B, u % B
        slot_b, slot_a = h % NB, u % NA
        head = pl.ds(_aligned(h * DH, DH), DH)
        group = pl.ds(_aligned(g * (REP * DH), REP * DH), REP * DH)

        xb = x_buf[1, pl.ds(b0, UB)].reshape(UB * SQ, D)
        qb = (_mm(xb, wq_buf[1, :, head]) * QSCALE).astype(bf16)
        qa = (_mm(x_buf[0, ba], wq_buf[0, :, group]) * QSCALE).astype(bf16)
        s_b = jnp.concatenate(
            [_mm_nt(qb[i * SQ:(i + 1) * SQ], load_piece(piece_b(slot_b, 0, b0 + i))) for i in range(UB)],
            axis=0)
        s_a = _mm_nt(jnp.concatenate([qa[:, j * DH:(j + 1) * DH] for j in range(REP)], axis=0),
                     load_piece(piece_a(slot_a, 0)))

        e, r = _softmax_parts(s_b)
        o_b = jnp.concatenate(
            [(_mm(e[i * SQ:(i + 1) * SQ], load_piece(piece_b(slot_b, 1, b0 + i)))
              * r[i * SQ:(i + 1) * SQ]).astype(bf16) for i in range(UB)], axis=0)
        e, r = _softmax_parts(s_a)
        o = (_mm(e, load_piece(piece_a(slot_a, 1))) * r).astype(bf16)
        o_a = jnp.concatenate([o[j * SQ:(j + 1) * SQ] for j in range(REP)], axis=1)

        acc[pl.ds(_aligned(b0 * SQ, UB * SQ), UB * SQ), D:] += _mm(o_b, wo_buf[1, head, :])
        acc[pl.ds(_aligned(ba * SQ, SQ), SQ), :D] += _mm(o_a, wo_buf[0, group, :])

    _start([(x.at[b], x_buf.at[part, b], pro_sem.at[0]) for b in range(B) for part, x in enumerate((ax, bx))])
    lax.fori_loop(0, 32, start_weight_reads, 0)
    lax.fori_loop(0, DIST, start_unit_reads, 0)
    acc[...] = jnp.zeros(acc.shape, jnp.float32)
    _wait_total(x_buf, pro_sem.at[0])
    _wait_total(wq_buf, pro_sem.at[1])
    _wait_total(wo_buf, pro_sem.at[2])

    def unit(u, carry):
        h, q = u // UPH, u % UPH

        @pl.when(u < T0)
        def _():
            start_unit_reads(u + DIST, 0)

        @pl.when(u >= T0)
        def _():
            @pl.when(u + DIST < NU)
            def _():
                _start(copies_gqa(u + DIST))

            lax.fori_loop(halves_before(u), halves_before(u + 1), start_half_unit_reads, 0)

        @pl.when(jnp.logical_and(q == 0, u < NMAIN))
        def _():
            _wait_total(kv_buf.at[pl.ds(piece_b(h % NB, 0, 0), 2 * B)], kv_sem.at[h % NB])

        @pl.when(u >= NMAIN)
        def _():
            for kv in range(2):
                _wait_total(kv_buf.at[pl.ds(piece_b(h % NB, kv, q * UB), UB)], kv_sem.at[NB + NA + u - NMAIN])

        _wait_total(kv_buf.at[pl.ds(piece_a(u % NA, 0), 2)], kv_sem.at[NB + u % NA])

        @pl.when(u == NU - 1)
        def _():
            lax.fori_loop(0, UPH - 1, start_writes, 0)

        compute_unit(u)

        @pl.when(h == HQ - 1)
        def _():
            rows = pl.ds(_aligned(q * (UB * SQ), UB * SQ), UB * SQ)
            stage[pl.ds(q * UB, UB)] = acc[rows, :].astype(bf16).reshape(UB, SQ, 2 * D)

        return carry

    lax.fori_loop(0, NU, unit, 0)
    start_writes(UPH - 1, 0)
    _wait_total(stage, out_sem)


@jax.jit
def pallas_concat_heads__gqa_block_cached__mha_block_cached__near_ridge_kernel(
    A_x: jax.Array,
    A_k_cache: jax.Array,
    A_v_cache: jax.Array,
    A_wq: jax.Array,
    A_wo: jax.Array,
    B_x: jax.Array,
    B_k_cache: jax.Array,
    B_v_cache: jax.Array,
    B_wq: jax.Array,
    B_wo: jax.Array,
):
    bf16 = jnp.bfloat16
    return pl.pallas_call(
        _kernel,
        out_shape=jax.ShapeDtypeStruct((B, SQ, 2 * D), bf16),
        in_specs=[pl.BlockSpec(memory_space=pl.ANY)] * 10,
        out_specs=pl.BlockSpec(memory_space=pl.ANY),
        scratch_shapes=[
            pltpu.VMEM((2, B, SQ, D), bf16),
            pltpu.VMEM((2, D, HQ * DH), bf16),
            pltpu.VMEM((2, HQ * DH, D), bf16),
            pltpu.VMEM((NB * 2 * B + NA * 2, SK, DH), bf16),
            pltpu.VMEM((ROWS, 2 * D), jnp.float32),
            pltpu.VMEM((B, SQ, 2 * D), bf16),
            pltpu.SemaphoreType.DMA((NB + NA + UPH * LAST_HEADS,)),
            pltpu.SemaphoreType.DMA((3,)),
            pltpu.SemaphoreType.DMA(()),
        ],
        compiler_params=pltpu.CompilerParams(
            vmem_limit_bytes=64 * 1024 * 1024,
            disable_bounds_checks=True,
        ),
    )(A_x, A_k_cache, A_v_cache, A_wq, A_wo, B_x, B_k_cache, B_v_cache, B_wq, B_wo)
```

```python
import math

import jax
import jax.numpy as jnp
from jax import lax
import jax.experimental.pallas as pl
import jax.experimental.pallas.tpu as pltpu

B, SQ, D = 16, 32, 512
HQ, SK, DH = 32, 512, 128
REP = 4
ROWS = B * SQ
QSCALE = (DH ** -0.5) * math.log2(math.e)

CH = 128
NCH = SK // CH
UB = 4
UPH = B // UB
NU = HQ * UPH

DIST = 7
LAST_HEADS = 2
DIST_END = 3
NA = DIST + 1
NB = (DIST + UPH - 1) // UPH + 1
NMAIN = NU - UPH * LAST_HEADS
T0 = NMAIN - DIST
NHALF = 2 * UPH * LAST_HEADS
TEND = NU - 1 - DIST_END
NSLOW = 2 * (TEND - T0 + 1) - NHALF
BATCH_ORDER = tuple(range(0, B, 2)) + tuple(range(1, B, 2))


def _aligned(x, n):
    return x if isinstance(x, int) else pl.multiple_of(x, n)


def _start(copies):
    for n, (src, dst, sem) in enumerate(copies):
        pltpu.make_async_copy(src, dst, sem).start(priority=n % 2)


def _wait_filled(buf, sem):
    pltpu.make_async_copy(buf, buf, sem).wait()


def _mm(a, b):
    return jnp.dot(a, b, preferred_element_type=jnp.float32)


def _mm_nt(a, b):
    return lax.dot_general(a, b, (((1,), (1,)), ((), ())), preferred_element_type=jnp.float32)


def _softmax_parts(s):
    e = jnp.exp2(s - jnp.max(s, axis=1, keepdims=True))
    return e.astype(jnp.bfloat16), 1.0 / jnp.sum(e, axis=1, keepdims=True)


def _kernel(ax, ak, av, awq, awo, bx, bk, bv, bwq, bwo, out,
            x_buf, wq_buf, wo_buf, kv_buf, q_words, acc, stage, kv_sem, pro_sem, out_sem):
    bf16 = jnp.bfloat16
    kv_words = kv_buf.bitcast(jnp.uint32)

    def piece_mha(h, b, kv):
        return ((h % NB) * B + b) * 2 + kv

    def piece_gqa(n, kv):
        return NB * B * 2 + (n % NA) * 2 + kv

    def load_piece(i):
        return pltpu.bitcast(kv_words[i], bf16)

    def copies_gqa(n):
        g, b = n // B, n % B
        return [(src.at[b, g, pl.ds(s * CH, CH)],
                 kv_buf.at[piece_gqa(n, kv), pl.ds(s * CH, CH)],
                 kv_sem.at[NB + n % NA])
                for s in range(NCH) for kv, src in enumerate((ak, av))]

    def copies_mha(n):
        h = n // UPH
        keys = pl.ds(_aligned((n % UPH) * CH, CH), CH)
        return [(src.at[b, h, keys], kv_buf.at[piece_mha(h, b, kv), keys], kv_sem.at[h % NB])
                for kv, src in enumerate((bk, bv)) for b in BATCH_ORDER]

    def start_unit_reads(n, carry):
        gqa, mha = copies_gqa(n), copies_mha(n)
        copies = []
        for i in range(4):
            copies += mha[8 * i:8 * i + 8] + gqa[2 * i:2 * i + 2]
        _start(copies)
        return carry

    def start_half_unit_reads(i, carry):
        j = i // 2
        h, b0 = HQ - LAST_HEADS + j // UPH, (j % UPH) * UB
        copies = []
        for s in range(NCH // 2):
            keys = pl.ds(_aligned(((i % 2) * (NCH // 2) + s) * CH, CH), CH)
            copies += [(src.at[b0 + b, h, keys], kv_buf.at[piece_mha(h, b0 + b, kv), keys],
                        kv_sem.at[NB + NA + j])
                       for kv, src in enumerate((bk, bv)) for b in range(UB)]
        _start(copies)
        return carry

    def start_weight_reads(i, carry):
        copies_q, copies_o = [], []
        for j in range(4):
            n = j * 32 + i
            rows, cols = pl.ds(_aligned((n // 2) * 8, 8), 8), pl.ds(_aligned((n % 2) * 2048, 2048), 2048)
            copies_q += [(w.at[rows, cols], wq_buf.at[part, rows, cols], pro_sem.at[1])
                         for part, w in enumerate((awq, bwq))]
            rows = pl.ds(_aligned(n * 32, 32), 32)
            copies_o += [(w.at[rows], wo_buf.at[part, rows], pro_sem.at[2])
                         for part, w in enumerate((awo, bwo))]
        _start(copies_q)
        _start(copies_o)
        return carry

    def start_writes(q):
        _start([(stage.at[b, pl.ds(j * 16, 16)], out.at[b, pl.ds(j * 16, 16)], out_sem)
                for j in range(SQ // 16) for b in range(q * UB, (q + 1) * UB)])

    def wait_gqa(u):
        _wait_filled(kv_buf.at[pl.ds(piece_gqa(u, 0), 2)], kv_sem.at[NB + u % NA])

    def wait_last_heads_unit(u):
        _wait_filled(kv_buf.at[pl.ds(piece_mha(u // UPH, (u % UPH) * UB, 0), 2 * UB)],
                     kv_sem.at[NB + NA + u - NMAIN])

    def halves_before(u):
        return jnp.clip(u - T0, 0, NSLOW) + jnp.clip(2 * (u - T0 - NSLOW), 0, NHALF - NSLOW)

    def project_q_gqa(u):
        group = pl.ds(_aligned((u // B) * (REP * DH), REP * DH), REP * DH)
        q = (_mm(x_buf[0, u % B], wq_buf[0, :, group]) * QSCALE).astype(bf16)
        q = jnp.concatenate([q[:, j * DH:(j + 1) * DH] for j in range(REP)], axis=0)
        q_words[0] = pltpu.bitcast(q, jnp.uint32)

    def project_q_mha(u):
        head = pl.ds(_aligned((u // UPH) * DH, DH), DH)
        x = x_buf[1, pl.ds((u % UPH) * UB, UB)].reshape(UB * SQ, D)
        q = (_mm(x, wq_buf[1, :, head]) * QSCALE).astype(bf16)
        q_words[1] = pltpu.bitcast(q, jnp.uint32)

    def compute_unit(u, project_next):
        h, b0 = u // UPH, (u % UPH) * UB
        g, ba = u // B, u % B
        q_a = pltpu.bitcast(q_words[0], bf16)
        q_b = pltpu.bitcast(q_words[1], bf16)

        e_a, r_a = _softmax_parts(_mm_nt(q_a, load_piece(piece_gqa(u, 0))))
        e_b, r_b = _softmax_parts(jnp.concatenate(
            [_mm_nt(q_b[i * SQ:(i + 1) * SQ], load_piece(piece_mha(h, b0 + i, 0))) for i in range(UB)],
            axis=0))

        o_a = (_mm(e_a, load_piece(piece_gqa(u, 1))) * r_a).astype(bf16)
        o_a = jnp.concatenate([o_a[j * SQ:(j + 1) * SQ] for j in range(REP)], axis=1)
        if project_next:
            project_q_mha(u + 1)
        o_b = jnp.concatenate(
            [(_mm(e_b[i * SQ:(i + 1) * SQ], load_piece(piece_mha(h, b0 + i, 1)))
              * r_b[i * SQ:(i + 1) * SQ]).astype(bf16) for i in range(UB)], axis=0)

        rows = pl.ds(_aligned(ba * SQ, SQ), SQ)
        group = pl.ds(_aligned(g * (REP * DH), REP * DH), REP * DH)
        res = acc[rows, :D] + _mm(o_a, wo_buf[0, group, :])
        if project_next:
            acc[rows, :D] = res
        stage[ba, :, :D] = res.astype(bf16)

        rows = pl.ds(_aligned(b0 * SQ, UB * SQ), UB * SQ)
        res = acc[rows, D:] + _mm(o_b, wo_buf[1, pl.ds(_aligned(h * DH, DH), DH), :])
        if project_next:
            acc[rows, D:] = res
        stage[pl.ds(b0, UB), :, D:] = res.astype(bf16).reshape(UB, SQ, D)

        if project_next:
            project_q_gqa(u + 1)

    _start([(x.at[b], x_buf.at[part, b], pro_sem.at[0]) for b in range(B) for part, x in enumerate((ax, bx))])
    lax.fori_loop(0, 32, start_weight_reads, 0)
    lax.fori_loop(0, DIST, start_unit_reads, 0)
    acc[...] = jnp.zeros(acc.shape, jnp.float32)
    _wait_filled(x_buf, pro_sem.at[0])
    _wait_filled(wq_buf, pro_sem.at[1])
    _wait_filled(wo_buf, pro_sem.at[2])
    project_q_mha(0)
    project_q_gqa(0)

    def unit(u, carry):
        h = u // UPH

        @pl.when(u < T0)
        def _():
            start_unit_reads(u + DIST, 0)

        @pl.when(u >= T0)
        def _():
            @pl.when(u + DIST < NU)
            def _():
                _start(copies_gqa(u + DIST))

            lax.fori_loop(halves_before(u), halves_before(u + 1), start_half_unit_reads, 0)

        @pl.when(jnp.logical_and(u % UPH == 0, u < NMAIN))
        def _():
            _wait_filled(kv_buf.at[pl.ds(piece_mha(h, 0, 0), 2 * B)], kv_sem.at[h % NB])

        @pl.when(u >= NMAIN)
        def _():
            wait_last_heads_unit(u)

        wait_gqa(u)

        @pl.when(u == NU - 2)
        def _():
            start_writes(0)

        compute_unit(u, True)
        return carry

    lax.fori_loop(0, NU - 1, unit, 0)

    wait_gqa(NU - 1)
    wait_last_heads_unit(NU - 1)
    for q in range(1, UPH - 1):
        start_writes(q)
    compute_unit(NU - 1, False)
    start_writes(UPH - 1)
    pltpu.make_async_copy(stage, out, out_sem).wait()


@jax.jit
def pallas_concat_heads__gqa_block_cached__mha_block_cached__near_ridge_kernel(
    A_x: jax.Array,
    A_k_cache: jax.Array,
    A_v_cache: jax.Array,
    A_wq: jax.Array,
    A_wo: jax.Array,
    B_x: jax.Array,
    B_k_cache: jax.Array,
    B_v_cache: jax.Array,
    B_wq: jax.Array,
    B_wo: jax.Array,
):
    bf16 = jnp.bfloat16
    return pl.pallas_call(
        _kernel,
        out_shape=jax.ShapeDtypeStruct((B, SQ, 2 * D), bf16),
        in_specs=[pl.BlockSpec(memory_space=pl.ANY)] * 10,
        out_specs=pl.BlockSpec(memory_space=pl.ANY),
        scratch_shapes=[
            pltpu.VMEM((2, B, SQ, D), bf16),
            pltpu.VMEM((2, D, HQ * DH), bf16),
            pltpu.VMEM((2, HQ * DH, D), bf16),
            pltpu.VMEM((NB * B * 2 + NA * 2, SK, DH), bf16),
            pltpu.VMEM((2, UB * SQ // 2, DH), jnp.uint32),
            pltpu.VMEM((ROWS, 2 * D), jnp.float32),
            pltpu.VMEM((B, SQ, 2 * D), bf16),
            pltpu.SemaphoreType.DMA((NB + NA + UPH * LAST_HEADS,)),
            pltpu.SemaphoreType.DMA((3,)),
            pltpu.SemaphoreType.DMA(()),
        ],
        compiler_params=pltpu.CompilerParams(
            vmem_limit_bytes=64 * 1024 * 1024,
            disable_bounds_checks=True,
            disable_semaphore_checks=True,
        ),
    )(A_x, A_k_cache, A_v_cache, A_wq, A_wo, B_x, B_k_cache, B_v_cache, B_wq, B_wo)
```

```python
import math

import jax
import jax.numpy as jnp
from jax import lax
import jax.experimental.pallas as pl
import jax.experimental.pallas.tpu as pltpu

B, SQ, D = 16, 32, 512
HQ, SK, DH = 32, 512, 128
REP = 4
ROWS = B * SQ
QSCALE = (DH ** -0.5) * math.log2(math.e)

CH = 128
NCH = SK // CH
UB = 4
UPH = B // UB
NU = HQ * UPH

DIST = 7
LAST_HEADS = 2
DIST_END = 3
NA = DIST + 1
NB = (DIST + UPH - 1) // UPH + 1
NMAIN = NU - UPH * LAST_HEADS
T0 = NMAIN - DIST
NHALF = 2 * UPH * LAST_HEADS
TEND = NU - 1 - DIST_END
NSLOW = 2 * (TEND - T0 + 1) - NHALF
BATCH_ORDER = tuple(range(0, B, 2)) + tuple(range(1, B, 2))


def _aligned(x, n):
    return x if isinstance(x, int) else pl.multiple_of(x, n)


def _start(copies):
    for n, (src, dst, sem) in enumerate(copies):
        pltpu.make_async_copy(src, dst, sem).start(priority=n % 2)


def _wait_filled(buf, sem):
    pltpu.make_async_copy(buf, buf, sem).wait()


def _mm(a, b):
    return jnp.dot(a, b, preferred_element_type=jnp.float32)


def _mm_nt(a, b):
    return lax.dot_general(a, b, (((1,), (1,)), ((), ())), preferred_element_type=jnp.float32)


def _softmax_parts(s):
    e = jnp.exp2(s - jnp.max(s, axis=1, keepdims=True))
    return e.astype(jnp.bfloat16), 1.0 / jnp.sum(e, axis=1, keepdims=True)


def _kernel(ax, ak, av, awq, awo, bx, bk, bv, bwq, bwo, out,
            x_buf, wq_buf, wo_buf, kv_buf, q_buf, acc, stage, kv_sem, pro_sem, out_sem):
    bf16 = jnp.bfloat16

    def piece_mha(h, b, kv):
        return ((h % NB) * B + b) * 2 + kv

    def piece_gqa(n, kv):
        return NB * B * 2 + (n % NA) * 2 + kv

    def copies_gqa(n):
        g, b = n // B, n % B
        return [(src.at[b, g, pl.ds(s * CH, CH)],
                 kv_buf.at[piece_gqa(n, kv), pl.ds(s * CH, CH)],
                 kv_sem.at[NB + n % NA])
                for s in range(NCH) for kv, src in enumerate((ak, av))]

    def copies_mha(n):
        h = n // UPH
        keys = pl.ds(_aligned((n % UPH) * CH, CH), CH)
        return [(src.at[b, h, keys], kv_buf.at[piece_mha(h, b, kv), keys], kv_sem.at[h % NB])
                for kv, src in enumerate((bk, bv)) for b in BATCH_ORDER]

    def start_unit_reads(n, carry):
        gqa, mha = copies_gqa(n), copies_mha(n)
        copies = []
        for i in range(4):
            copies += mha[8 * i:8 * i + 8] + gqa[2 * i:2 * i + 2]
        _start(copies)
        return carry

    def start_half_unit_reads(i, carry):
        j = i // 2
        h, b0 = HQ - LAST_HEADS + j // UPH, (j % UPH) * UB
        copies = []
        for s in range(NCH // 2):
            keys = pl.ds(_aligned(((i % 2) * (NCH // 2) + s) * CH, CH), CH)
            copies += [(src.at[b0 + b, h, keys], kv_buf.at[piece_mha(h, b0 + b, kv), keys],
                        kv_sem.at[NB + NA + j])
                       for kv, src in enumerate((bk, bv)) for b in range(UB)]
        _start(copies)
        return carry

    def start_weight_reads(i, carry):
        copies_q, copies_o = [], []
        for j in range(4):
            n = j * 32 + i
            rows, cols = pl.ds(_aligned((n // 2) * 8, 8), 8), pl.ds(_aligned((n % 2) * 2048, 2048), 2048)
            copies_q += [(w.at[rows, cols], wq_buf.at[part, rows, cols], pro_sem.at[1])
                         for part, w in enumerate((awq, bwq))]
            rows = pl.ds(_aligned(n * 32, 32), 32)
            copies_o += [(w.at[rows], wo_buf.at[part, rows], pro_sem.at[2])
                         for part, w in enumerate((awo, bwo))]
        _start(copies_q)
        _start(copies_o)
        return carry

    def start_writes(q):
        _start([(stage.at[b, pl.ds(j * 16, 16)], out.at[b, pl.ds(j * 16, 16)], out_sem)
                for j in range(SQ // 16) for b in range(q * UB, (q + 1) * UB)])

    def wait_gqa(u):
        _wait_filled(kv_buf.at[pl.ds(piece_gqa(u, 0), 2)], kv_sem.at[NB + u % NA])

    def wait_last_heads_unit(u):
        _wait_filled(kv_buf.at[pl.ds(piece_mha(u // UPH, (u % UPH) * UB, 0), 2 * UB)],
                     kv_sem.at[NB + NA + u - NMAIN])

    def halves_before(u):
        return jnp.clip(u - T0, 0, NSLOW) + jnp.clip(2 * (u - T0 - NSLOW), 0, NHALF - NSLOW)

    def project_q_gqa(u):
        group = pl.ds(_aligned((u // B) * (REP * DH), REP * DH), REP * DH)
        q = (_mm(x_buf[0, u % B], wq_buf[0, :, group]) * QSCALE).astype(bf16)
        q_buf[0] = jnp.concatenate([q[:, j * DH:(j + 1) * DH] for j in range(REP)], axis=0)

    def project_q_mha(u):
        head = pl.ds(_aligned((u // UPH) * DH, DH), DH)
        x = x_buf[1, pl.ds((u % UPH) * UB, UB)].reshape(UB * SQ, D)
        q_buf[1] = (_mm(x, wq_buf[1, :, head]) * QSCALE).astype(bf16)

    def compute_unit(u, project_next):
        h, b0 = u // UPH, (u % UPH) * UB
        g, ba = u // B, u % B
        q_a = q_buf[0]
        q_b = q_buf[1]

        e_a, r_a = _softmax_parts(_mm_nt(q_a, kv_buf[piece_gqa(u, 0)]))
        e_b, r_b = _softmax_parts(jnp.concatenate(
            [_mm_nt(q_b[i * SQ:(i + 1) * SQ], kv_buf[piece_mha(h, b0 + i, 0)]) for i in range(UB)],
            axis=0))

        o_a = (_mm(e_a, kv_buf[piece_gqa(u, 1)]) * r_a).astype(bf16)
        o_a = jnp.concatenate([o_a[j * SQ:(j + 1) * SQ] for j in range(REP)], axis=1)
        if project_next:
            project_q_mha(u + 1)
        o_b = jnp.concatenate(
            [(_mm(e_b[i * SQ:(i + 1) * SQ], kv_buf[piece_mha(h, b0 + i, 1)])
              * r_b[i * SQ:(i + 1) * SQ]).astype(bf16) for i in range(UB)], axis=0)

        rows = pl.ds(_aligned(ba * SQ, SQ), SQ)
        group = pl.ds(_aligned(g * (REP * DH), REP * DH), REP * DH)
        res = acc[rows, :D] + _mm(o_a, wo_buf[0, group, :])
        if project_next:
            acc[rows, :D] = res
        stage[ba, :, :D] = res.astype(bf16)

        rows = pl.ds(_aligned(b0 * SQ, UB * SQ), UB * SQ)
        res = acc[rows, D:] + _mm(o_b, wo_buf[1, pl.ds(_aligned(h * DH, DH), DH), :])
        if project_next:
            acc[rows, D:] = res
        stage[pl.ds(b0, UB), :, D:] = res.astype(bf16).reshape(UB, SQ, D)

        if project_next:
            project_q_gqa(u + 1)

    _start([(x.at[b], x_buf.at[part, b], pro_sem.at[0]) for b in range(B) for part, x in enumerate((ax, bx))])
    lax.fori_loop(0, 32, start_weight_reads, 0)
    lax.fori_loop(0, DIST, start_unit_reads, 0)
    acc[...] = jnp.zeros(acc.shape, jnp.float32)
    _wait_filled(x_buf, pro_sem.at[0])
    _wait_filled(wq_buf, pro_sem.at[1])
    _wait_filled(wo_buf, pro_sem.at[2])
    project_q_mha(0)
    project_q_gqa(0)

    def unit(u, carry):
        h = u // UPH

        @pl.when(u < T0)
        def _():
            start_unit_reads(u + DIST, 0)

        @pl.when(u >= T0)
        def _():
            @pl.when(u + DIST < NU)
            def _():
                _start(copies_gqa(u + DIST))

            lax.fori_loop(halves_before(u), halves_before(u + 1), start_half_unit_reads, 0)

        @pl.when(jnp.logical_and(u % UPH == 0, u < NMAIN))
        def _():
            _wait_filled(kv_buf.at[pl.ds(piece_mha(h, 0, 0), 2 * B)], kv_sem.at[h % NB])

        @pl.when(u >= NMAIN)
        def _():
            wait_last_heads_unit(u)

        wait_gqa(u)

        @pl.when(u == NU - 2)
        def _():
            start_writes(0)

        compute_unit(u, True)
        return carry

    lax.fori_loop(0, NU - 1, unit, 0)

    wait_gqa(NU - 1)
    wait_last_heads_unit(NU - 1)
    for q in range(1, UPH - 1):
        start_writes(q)
    compute_unit(NU - 1, False)
    start_writes(UPH - 1)
    pltpu.make_async_copy(stage, out, out_sem).wait()


@jax.jit
def pallas_concat_heads__gqa_block_cached__mha_block_cached__near_ridge_kernel(
    A_x: jax.Array,
    A_k_cache: jax.Array,
    A_v_cache: jax.Array,
    A_wq: jax.Array,
    A_wo: jax.Array,
    B_x: jax.Array,
    B_k_cache: jax.Array,
    B_v_cache: jax.Array,
    B_wq: jax.Array,
    B_wo: jax.Array,
):
    bf16 = jnp.bfloat16
    return pl.pallas_call(
        _kernel,
        out_shape=jax.ShapeDtypeStruct((B, SQ, 2 * D), bf16),
        in_specs=[pl.BlockSpec(memory_space=pl.ANY)] * 10,
        out_specs=pl.BlockSpec(memory_space=pl.ANY),
        scratch_shapes=[
            pltpu.VMEM((2, B, SQ, D), bf16),
            pltpu.VMEM((2, D, HQ * DH), bf16),
            pltpu.VMEM((2, HQ * DH, D), bf16),
            pltpu.VMEM((NB * B * 2 + NA * 2, SK, DH), bf16),
            pltpu.VMEM((2, UB * SQ, DH), bf16),
            pltpu.VMEM((ROWS, 2 * D), jnp.float32),
            pltpu.VMEM((B, SQ, 2 * D), bf16),
            pltpu.SemaphoreType.DMA((NB + NA + UPH * LAST_HEADS,)),
            pltpu.SemaphoreType.DMA((3,)),
            pltpu.SemaphoreType.DMA(()),
        ],
        compiler_params=pltpu.CompilerParams(
            vmem_limit_bytes=64 * 1024 * 1024,
            disable_bounds_checks=True,
            disable_semaphore_checks=True,
        ),
    )(A_x, A_k_cache, A_v_cache, A_wq, A_wo, B_x, B_k_cache, B_v_cache, B_wq, B_wo)
```

```python
import math

import jax
import jax.numpy as jnp
from jax import lax
import jax.experimental.pallas as pl
import jax.experimental.pallas.tpu as pltpu

B, SQ, D = 16, 32, 512
HQ, SK, DH = 32, 512, 128
REP = 4
ROWS = B * SQ
QSCALE = (DH ** -0.5) * math.log2(math.e)

CH = 128
NCH = SK // CH
UB = 4
UPH = B // UB
NU = HQ * UPH

DIST = 6
DIST_GQA = DIST + B - 3
NA = 3
NB = (DIST + UPH - 1) // UPH + 1
LAST_HEADS = 4
DIST_END = 3
NMAIN = NU - UPH * LAST_HEADS
NHALF = 2 * UPH * LAST_HEADS
T0 = NMAIN - DIST
TEND = NU - 1 - DIST_END
assert T0 + DIST_GQA <= NU
BATCH_ORDER = tuple(range(B - 1, 0, -2)) + tuple(range(B - 2, -1, -2))


def _aligned(x, n):
    return x if isinstance(x, int) else pl.multiple_of(x, n)


def _start(copies):
    for n, (src, dst, sem) in enumerate(copies):
        pltpu.make_async_copy(src, dst, sem).start(priority=n % 2)


def _wait_filled(buf, sem):
    pltpu.make_async_copy(buf, buf, sem).wait()


def _mm(a, b):
    return jnp.dot(a, b, preferred_element_type=jnp.float32)


def _mm_nt(a, b):
    return lax.dot_general(a, b, (((1,), (1,)), ((), ())), preferred_element_type=jnp.float32)


def _softmax_parts(s):
    e = jnp.exp2(s - jnp.max(s, axis=1, keepdims=True))
    return e.astype(jnp.bfloat16), 1.0 / jnp.sum(e, axis=1, keepdims=True)


def _kernel(ax, ak, av, awq, awo, bx, bk, bv, bwq, bwo, out,
            x_buf, wq_buf, wo_buf, kv_buf, q_buf, acc, stage, kv_sem, pro_sem, out_sem):
    bf16 = jnp.bfloat16

    def piece_mha(h, b, kv):
        return ((h % NB) * B + b) * 2 + kv

    def piece_gqa(g, b, kv):
        return ((NB + g % NA) * B + b) * 2 + kv

    def copies_gqa(n):
        g, p = n // B, n % B
        keys = pl.ds(_aligned((p // 4) * CH, CH), CH)
        batches = [(p % 4) * 4 + i for i in range(4)]
        return [(src.at[b, g, keys], kv_buf.at[piece_gqa(g, b, kv), keys], kv_sem.at[NB + g % NA])
                for kv, src in enumerate((ak, av)) for b in batches]

    def copies_mha(n):
        h = n // UPH
        keys = pl.ds(_aligned((n % UPH) * CH, CH), CH)
        return [(src.at[b, h, keys], kv_buf.at[piece_mha(h, b, kv), keys], kv_sem.at[h % NB])
                for kv, src in enumerate((bk, bv)) for b in BATCH_ORDER]

    def start_gqa_reads(n, carry):
        _start(copies_gqa(n))
        return carry

    def start_reads(n, carry):
        _start(copies_gqa(n + DIST_GQA - DIST) + copies_mha(n))
        return carry

    def start_half_unit_reads(i, carry):
        j = i // 2
        h, b0 = HQ - LAST_HEADS + j // UPH, (j % UPH) * UB
        copies = []
        for s in range(NCH // 2):
            keys = pl.ds(_aligned(((i % 2) * (NCH // 2) + s) * CH, CH), CH)
            copies += [(src.at[b0 + b, h, keys], kv_buf.at[piece_mha(h, b0 + b, kv), keys],
                        kv_sem.at[NB + NA + j])
                       for kv, src in enumerate((bk, bv)) for b in range(UB)]
        _start(copies)
        return carry

    def start_weight_reads(i, carry):
        copies_q, copies_o = [], []
        for j in range(4):
            n = j * 32 + i
            rows, cols = pl.ds(_aligned((n // 2) * 8, 8), 8), pl.ds(_aligned((n % 2) * 2048, 2048), 2048)
            copies_q += [(w.at[rows, cols], wq_buf.at[part, rows, cols], pro_sem.at[1])
                         for part, w in enumerate((awq, bwq))]
            rows = pl.ds(_aligned(n * 32, 32), 32)
            copies_o += [(w.at[rows], wo_buf.at[part, rows], pro_sem.at[2])
                         for part, w in enumerate((awo, bwo))]
        _start(copies_q)
        _start(copies_o)
        return carry

    def start_writes(q):
        _start([(stage.at[b, pl.ds(j * 16, 16)], out.at[b, pl.ds(j * 16, 16)], out_sem)
                for j in range(SQ // 16) for b in range(q * UB, (q + 1) * UB)])

    def wait_last_heads_unit(u):
        _wait_filled(kv_buf.at[pl.ds(piece_mha(u // UPH, (u % UPH) * UB, 0), 2 * UB)],
                     kv_sem.at[NB + NA + u - NMAIN])

    def halves_before(u):
        return jnp.minimum((u - T0) * NHALF // (TEND - T0 + 1), NHALF)

    def project_q_gqa(u):
        group = pl.ds(_aligned((u // B) * (REP * DH), REP * DH), REP * DH)
        q = (_mm(x_buf[0, u % B], wq_buf[0, :, group]) * QSCALE).astype(bf16)
        q_buf[0] = jnp.concatenate([q[:, j * DH:(j + 1) * DH] for j in range(REP)], axis=0)

    def project_q_mha(u):
        head = pl.ds(_aligned((u // UPH) * DH, DH), DH)
        x = x_buf[1, pl.ds((u % UPH) * UB, UB)].reshape(UB * SQ, D)
        q_buf[1] = (_mm(x, wq_buf[1, :, head]) * QSCALE).astype(bf16)

    def compute_unit(u, project_next):
        h, b0 = u // UPH, (u % UPH) * UB
        g, ba = u // B, u % B
        q_a = q_buf[0]
        q_b = q_buf[1]

        e_a, r_a = _softmax_parts(_mm_nt(q_a, kv_buf[piece_gqa(g, ba, 0)]))
        e_b, r_b = _softmax_parts(jnp.concatenate(
            [_mm_nt(q_b[i * SQ:(i + 1) * SQ], kv_buf[piece_mha(h, b0 + i, 0)]) for i in range(UB)],
            axis=0))

        o_a = (_mm(e_a, kv_buf[piece_gqa(g, ba, 1)]) * r_a).astype(bf16)
        o_a = jnp.concatenate([o_a[j * SQ:(j + 1) * SQ] for j in range(REP)], axis=1)
        if project_next:
            project_q_mha(u + 1)
        o_b = jnp.concatenate(
            [(_mm(e_b[i * SQ:(i + 1) * SQ], kv_buf[piece_mha(h, b0 + i, 1)])
              * r_b[i * SQ:(i + 1) * SQ]).astype(bf16) for i in range(UB)], axis=0)

        rows = pl.ds(_aligned(ba * SQ, SQ), SQ)
        group = pl.ds(_aligned(g * (REP * DH), REP * DH), REP * DH)
        res = acc[rows, :D] + _mm(o_a, wo_buf[0, group, :])
        if project_next:
            acc[rows, :D] = res
        stage[ba, :, :D] = res.astype(bf16)

        rows = pl.ds(_aligned(b0 * SQ, UB * SQ), UB * SQ)
        res = acc[rows, D:] + _mm(o_b, wo_buf[1, pl.ds(_aligned(h * DH, DH), DH), :])
        if project_next:
            acc[rows, D:] = res
        stage[pl.ds(b0, UB), :, D:] = res.astype(bf16).reshape(UB, SQ, D)

        if project_next:
            project_q_gqa(u + 1)

    _start([(x.at[b], x_buf.at[part, b], pro_sem.at[0]) for b in range(B) for part, x in enumerate((ax, bx))])
    lax.fori_loop(0, 32, start_weight_reads, 0)
    lax.fori_loop(0, DIST_GQA - DIST, start_gqa_reads, 0)
    lax.fori_loop(0, DIST, start_reads, 0)
    acc[...] = jnp.zeros(acc.shape, jnp.float32)
    _wait_filled(x_buf, pro_sem.at[0])
    _wait_filled(wq_buf, pro_sem.at[1])
    _wait_filled(wo_buf, pro_sem.at[2])
    project_q_mha(0)
    project_q_gqa(0)

    def unit(u, carry):
        h, g = u // UPH, u // B

        @pl.when(u < T0)
        def _():
            start_reads(u + DIST, 0)

        @pl.when(u >= T0)
        def _():
            @pl.when(u + DIST_GQA < NU)
            def _():
                start_gqa_reads(u + DIST_GQA, 0)

            lax.fori_loop(halves_before(u), halves_before(u + 1), start_half_unit_reads, 0)

        @pl.when(jnp.logical_and(u % UPH == 0, u < NMAIN))
        def _():
            _wait_filled(kv_buf.at[pl.ds(piece_mha(h, 0, 0), 2 * B)], kv_sem.at[h % NB])

        @pl.when(u >= NMAIN)
        def _():
            wait_last_heads_unit(u)

        @pl.when(u % B == 0)
        def _():
            _wait_filled(kv_buf.at[pl.ds(piece_gqa(g, 0, 0), 2 * B)], kv_sem.at[NB + g % NA])

        @pl.when(u == NU - 2)
        def _():
            start_writes(0)

        compute_unit(u, True)
        return carry

    lax.fori_loop(0, NU - 1, unit, 0)

    wait_last_heads_unit(NU - 1)
    for q in range(1, UPH - 1):
        start_writes(q)
    compute_unit(NU - 1, False)
    start_writes(UPH - 1)
    pltpu.make_async_copy(stage, out, out_sem).wait()


@jax.jit
def pallas_concat_heads__gqa_block_cached__mha_block_cached__near_ridge_kernel(
    A_x: jax.Array,
    A_k_cache: jax.Array,
    A_v_cache: jax.Array,
    A_wq: jax.Array,
    A_wo: jax.Array,
    B_x: jax.Array,
    B_k_cache: jax.Array,
    B_v_cache: jax.Array,
    B_wq: jax.Array,
    B_wo: jax.Array,
):
    bf16 = jnp.bfloat16
    return pl.pallas_call(
        _kernel,
        out_shape=jax.ShapeDtypeStruct((B, SQ, 2 * D), bf16),
        in_specs=[pl.BlockSpec(memory_space=pl.ANY)] * 10,
        out_specs=pl.BlockSpec(memory_space=pl.ANY),
        scratch_shapes=[
            pltpu.VMEM((2, B, SQ, D), bf16),
            pltpu.VMEM((2, D, HQ * DH), bf16),
            pltpu.VMEM((2, HQ * DH, D), bf16),
            pltpu.VMEM(((NB + NA) * B * 2, SK, DH), bf16),
            pltpu.VMEM((2, UB * SQ, DH), bf16),
            pltpu.VMEM((ROWS, 2 * D), jnp.float32),
            pltpu.VMEM((B, SQ, 2 * D), bf16),
            pltpu.SemaphoreType.DMA((NB + NA + UPH * LAST_HEADS,)),
            pltpu.SemaphoreType.DMA((3,)),
            pltpu.SemaphoreType.DMA(()),
        ],
        compiler_params=pltpu.CompilerParams(
            vmem_limit_bytes=64 * 1024 * 1024,
            disable_bounds_checks=True,
            disable_semaphore_checks=True,
        ),
    )(A_x, A_k_cache, A_v_cache, A_wq, A_wo, B_x, B_k_cache, B_v_cache, B_wq, B_wo)
```

```python
import math

import jax
import jax.numpy as jnp
from jax import lax
import jax.experimental.pallas as pl
import jax.experimental.pallas.tpu as pltpu

B, SQ, D = 16, 32, 512
HQ, SK, DH = 32, 512, 128
REP = 4
ROWS = B * SQ
QSCALE = (DH ** -0.5) * math.log2(math.e)

CH = 128
NCH = SK // CH
UB = 4
UPH = B // UB
NU = HQ * UPH

DIST = 6
DIST_GQA = DIST + B - 3
NA = 3
NB = (DIST + UPH - 1) // UPH + 1
LAST_HEADS = 4
DIST_END = 3
NMAIN = NU - UPH * LAST_HEADS
NHALF = 2 * UPH * LAST_HEADS
T0 = NMAIN - DIST
TEND = NU - 1 - DIST_END
assert T0 + DIST_GQA <= NU
BATCH_ORDER = tuple(range(B - 1, 0, -2)) + tuple(range(B - 2, -1, -2))


def _aligned(x, n):
    return x if isinstance(x, int) else pl.multiple_of(x, n)


def _start(copies):
    for n, (src, dst, sem) in enumerate(copies):
        pltpu.make_async_copy(src, dst, sem).start(priority=n % 2)


def _wait_filled(buf, sem):
    pltpu.make_async_copy(buf, buf, sem).wait()


def _mm(a, b):
    return jnp.dot(a, b, preferred_element_type=jnp.float32)


def _mm_nt(a, b):
    return lax.dot_general(a, b, (((1,), (1,)), ((), ())), preferred_element_type=jnp.float32)


def _softmax_parts(s):
    e = jnp.exp2(s - jnp.max(s, axis=1, keepdims=True))
    return e.astype(jnp.bfloat16), 1.0 / jnp.sum(e, axis=1, keepdims=True)


def _kernel(ax, ak, av, awq, awo, bx, bk, bv, bwq, bwo, out,
            x_buf, wq_buf, wo_buf, kv_buf, q_buf, acc, stage, kv_sem, pro_sem, out_sem):
    bf16 = jnp.bfloat16

    def piece_mha(h, b, kv):
        return ((h % NB) * B + b) * 2 + kv

    def piece_gqa(g, b, kv):
        return ((NB + g % NA) * B + b) * 2 + kv

    def copies_gqa(n):
        g, p = n // B, n % B
        keys = pl.ds(_aligned((p // 4) * CH, CH), CH)
        batches = [(p % 4) * 4 + i for i in range(4)]
        return [(src.at[b, g, keys], kv_buf.at[piece_gqa(g, b, kv), keys], kv_sem.at[NB + g % NA])
                for kv, src in enumerate((ak, av)) for b in batches]

    def copies_mha(n):
        h = n // UPH
        keys = pl.ds(_aligned((n % UPH) * CH, CH), CH)
        return [(src.at[b, h, keys], kv_buf.at[piece_mha(h, b, kv), keys], kv_sem.at[h % NB])
                for kv, src in enumerate((bk, bv)) for b in BATCH_ORDER]

    def start_gqa_reads(n, carry):
        _start(copies_gqa(n))
        return carry

    def start_reads(n, carry):
        _start(copies_gqa(n + DIST_GQA - DIST) + copies_mha(n))
        return carry

    def start_half_unit_reads(i, carry):
        j = i // 2
        h, b0 = HQ - LAST_HEADS + j // UPH, (j % UPH) * UB
        copies = []
        for s in range(NCH // 2):
            keys = pl.ds(_aligned(((i % 2) * (NCH // 2) + s) * CH, CH), CH)
            copies += [(src.at[b0 + b, h, keys], kv_buf.at[piece_mha(h, b0 + b, kv), keys],
                        kv_sem.at[NB + NA + j])
                       for kv, src in enumerate((bk, bv)) for b in range(UB)]
        _start(copies)
        return carry

    def start_weight_reads(i, carry):
        copies_q, copies_o = [], []
        for j in range(4):
            n = j * 32 + i
            rows, cols = pl.ds(_aligned((n // 2) * 8, 8), 8), pl.ds(_aligned((n % 2) * 2048, 2048), 2048)
            copies_q += [(w.at[rows, cols], wq_buf.at[part, rows, cols], pro_sem.at[1])
                         for part, w in enumerate((awq, bwq))]
            rows = pl.ds(_aligned(n * 32, 32), 32)
            copies_o += [(w.at[rows], wo_buf.at[part, rows], pro_sem.at[2])
                         for part, w in enumerate((awo, bwo))]
        _start(copies_q)
        _start(copies_o)
        return carry

    def start_writes(q):
        _start([(stage.at[b, pl.ds(j * 16, 16)], out.at[b, pl.ds(j * 16, 16)], out_sem)
                for j in range(SQ // 16) for b in range(q * UB, (q + 1) * UB)])

    def wait_last_heads_unit(u):
        _wait_filled(kv_buf.at[pl.ds(piece_mha(u // UPH, (u % UPH) * UB, 0), 2 * UB)],
                     kv_sem.at[NB + NA + u - NMAIN])

    def halves_before(u):
        return jnp.minimum((u - T0) * NHALF // (TEND - T0 + 1), NHALF)

    def project_q_gqa(u):
        group = pl.ds(_aligned((u // B) * (REP * DH), REP * DH), REP * DH)
        q = (_mm(x_buf[0, u % B], wq_buf[0, :, group]) * QSCALE).astype(bf16)
        q_buf[0] = jnp.concatenate([q[:, j * DH:(j + 1) * DH] for j in range(REP)], axis=0)

    def project_q_mha(u):
        head = pl.ds(_aligned((u // UPH) * DH, DH), DH)
        x = x_buf[1, pl.ds((u % UPH) * UB, UB)].reshape(UB * SQ, D)
        q_buf[1] = (_mm(x, wq_buf[1, :, head]) * QSCALE).astype(bf16)

    def compute_unit(u, last):
        h, b0 = u // UPH, (u % UPH) * UB
        g, ba = u // B, u % B
        q_a = q_buf[0]
        q_b = q_buf[1]

        e_a, r_a = _softmax_parts(_mm_nt(q_a, kv_buf[piece_gqa(g, ba, 0)]))
        e_b, r_b = _softmax_parts(jnp.concatenate(
            [_mm_nt(q_b[i * SQ:(i + 1) * SQ], kv_buf[piece_mha(h, b0 + i, 0)]) for i in range(UB)],
            axis=0))

        o_a = (_mm(e_a, kv_buf[piece_gqa(g, ba, 1)]) * r_a).astype(bf16)
        o_a = jnp.concatenate([o_a[j * SQ:(j + 1) * SQ] for j in range(REP)], axis=1)
        if not last:
            project_q_mha(u + 1)
        o_b = jnp.concatenate(
            [(_mm(e_b[i * SQ:(i + 1) * SQ], kv_buf[piece_mha(h, b0 + i, 1)])
              * r_b[i * SQ:(i + 1) * SQ]).astype(bf16) for i in range(UB)], axis=0)

        rows = pl.ds(_aligned(ba * SQ, SQ), SQ)
        group = pl.ds(_aligned(g * (REP * DH), REP * DH), REP * DH)
        res = acc[rows, :D] + _mm(o_a, wo_buf[0, group, :])
        if not last:
            acc[rows, :D] = res
        stage[ba, :, :D] = res.astype(bf16)

        rows = pl.ds(_aligned(b0 * SQ, UB * SQ), UB * SQ)
        res = acc[rows, D:] + _mm(o_b, wo_buf[1, pl.ds(_aligned(h * DH, DH), DH), :])
        if not last:
            acc[rows, D:] = res
        stage[pl.ds(b0, UB), :, D:] = res.astype(bf16).reshape(UB, SQ, D)

        if not last:
            project_q_gqa(u + 1)

    _start([(x.at[b], x_buf.at[part, b], pro_sem.at[0]) for b in range(B) for part, x in enumerate((ax, bx))])
    lax.fori_loop(0, 32, start_weight_reads, 0)
    lax.fori_loop(0, DIST_GQA - DIST, start_gqa_reads, 0)
    lax.fori_loop(0, DIST, start_reads, 0)
    acc[...] = jnp.zeros(acc.shape, jnp.float32)
    _wait_filled(x_buf, pro_sem.at[0])
    _wait_filled(wq_buf, pro_sem.at[1])
    _wait_filled(wo_buf, pro_sem.at[2])
    project_q_mha(0)
    project_q_gqa(0)

    def unit(u, carry):
        h, g = u // UPH, u // B

        @pl.when(u < T0)
        def _():
            start_reads(u + DIST, 0)

        @pl.when(u >= T0)
        def _():
            @pl.when(u + DIST_GQA < NU)
            def _():
                start_gqa_reads(u + DIST_GQA, 0)

            lax.fori_loop(halves_before(u), halves_before(u + 1), start_half_unit_reads, 0)

        @pl.when(jnp.logical_and(u % UPH == 0, u < NMAIN))
        def _():
            _wait_filled(kv_buf.at[pl.ds(piece_mha(h, 0, 0), 2 * B)], kv_sem.at[h % NB])

        @pl.when(u >= NMAIN)
        def _():
            wait_last_heads_unit(u)

        @pl.when(u % B == 0)
        def _():
            _wait_filled(kv_buf.at[pl.ds(piece_gqa(g, 0, 0), 2 * B)], kv_sem.at[NB + g % NA])

        @pl.when(u == NU - 2)
        def _():
            start_writes(0)

        compute_unit(u, last=False)
        return carry

    lax.fori_loop(0, NU - 1, unit, 0)

    wait_last_heads_unit(NU - 1)
    for q in range(1, UPH - 1):
        start_writes(q)
    compute_unit(NU - 1, last=True)
    start_writes(UPH - 1)
    pltpu.make_async_copy(stage, out, out_sem).wait()


@jax.jit
def pallas_concat_heads__gqa_block_cached__mha_block_cached__near_ridge_kernel(
    A_x: jax.Array,
    A_k_cache: jax.Array,
    A_v_cache: jax.Array,
    A_wq: jax.Array,
    A_wo: jax.Array,
    B_x: jax.Array,
    B_k_cache: jax.Array,
    B_v_cache: jax.Array,
    B_wq: jax.Array,
    B_wo: jax.Array,
):
    bf16 = jnp.bfloat16
    assert A_x.shape == B_x.shape == (B, SQ, D)
    assert A_k_cache.shape == A_v_cache.shape == (B, HQ // REP, SK, DH)
    assert B_k_cache.shape == B_v_cache.shape == (B, HQ, SK, DH)
    assert A_wq.shape == B_wq.shape == (D, HQ * DH)
    assert A_wo.shape == B_wo.shape == (HQ * DH, D)
    return pl.pallas_call(
        _kernel,
        out_shape=jax.ShapeDtypeStruct((B, SQ, 2 * D), bf16),
        in_specs=[pl.BlockSpec(memory_space=pl.ANY)] * 10,
        out_specs=pl.BlockSpec(memory_space=pl.ANY),
        scratch_shapes=[
            pltpu.VMEM((2, B, SQ, D), bf16),
            pltpu.VMEM((2, D, HQ * DH), bf16),
            pltpu.VMEM((2, HQ * DH, D), bf16),
            pltpu.VMEM(((NB + NA) * B * 2, SK, DH), bf16),
            pltpu.VMEM((2, UB * SQ, DH), bf16),
            pltpu.VMEM((ROWS, 2 * D), jnp.float32),
            pltpu.VMEM((B, SQ, 2 * D), bf16),
            pltpu.SemaphoreType.DMA((NB + NA + UPH * LAST_HEADS,)),
            pltpu.SemaphoreType.DMA((3,)),
            pltpu.SemaphoreType.DMA(()),
        ],
        compiler_params=pltpu.CompilerParams(
            vmem_limit_bytes=64 * 1024 * 1024,
            disable_bounds_checks=True,
            disable_semaphore_checks=True,
        ),
    )(A_x, A_k_cache, A_v_cache, A_wq, A_wo, B_x, B_k_cache, B_v_cache, B_wq, B_wo)
```
